```python
import os as _os
_os.environ.setdefault("JAX_PLATFORMS", "cpu")
import jax
import jax.numpy as jnp

def _softmax(x, axis=-1):
    return jax.nn.softmax(x, axis=axis)
def _gelu(x):
    return jax.nn.gelu(x, approximate=True)
def _silu(x):
    return jax.nn.silu(x)
def _sigmoid(x):
    return jax.nn.sigmoid(x)
def _layernorm(x, axis=-1, eps=1e-5):
    m = jnp.mean(x, axis=axis, keepdims=True)
    v = jnp.var(x, axis=axis, keepdims=True)
    return (x - m) / jnp.sqrt(v + eps)
def _scatter_add(tgt, idx, src, axis=0):
    return tgt.at[idx].add(src)
def _segment_sum(src, seg, n):
    return jax.ops.segment_sum(src, seg, n)
class _Rng:
    def __init__(self, key):
        self._k = key
    def _next(self):
        self._k, sub = jax.random.split(self._k)
        return sub
    def normal(self, shape):
        return jax.random.normal(self._next(), shape, dtype=jnp.bfloat16)
    def randint(self, lo, hi, shape):
        return jax.random.randint(self._next(), shape, lo, hi, dtype=jnp.int32)
    def uniform(self, shape, lo=0.0, hi=1.0):
        return jax.random.uniform(self._next(), shape, jnp.bfloat16, lo, hi)
    def permutation(self, n):
        return jax.random.permutation(self._next(), n)


kernel_name = 'concat_heads__sliding_local_dilated__sliding_block__prompt'

def setup_inputs():
    _rng = _Rng(jax.random.key(int.from_bytes(__import__("os").urandom(4), "little")))
    _w = (lambda a: (lambda t: t.astype(jnp.bfloat16) if jnp.issubdtype(t.dtype, jnp.floating) else t)(jnp.asarray(a)))
    def _A_setup():
        B, S, D = 1, 2048, 1024
        return {
            "x": _w((lambda *s: _rng.normal(s) * 0.2)(B, S, D)),
            "wqkv": _w((lambda *s: _rng.normal(s) * 0.2)(D, 3 * D)),
            "wo": _w((lambda *s: _rng.normal(s) * 0.05)(D, D)),
        }
    _A_in = _A_setup()

    def _B_setup():
        B, S, D = 1, 2048, 1024
        return {
            "x": _w((lambda *s: _rng.normal(s) * 0.2)(B, S, D)),
            "wqkv": _w((lambda *s: _rng.normal(s) * 0.2)(D, 3 * D)),
            "wo": _w((lambda *s: _rng.normal(s) * 0.05)(D, D)),
        }
    _B_in = _B_setup()

    return {
        "A_x": _A_in["x"],
        "A_wqkv": _A_in["wqkv"],
        "A_wo": _A_in["wo"],
        "B_x": _B_in["x"],
        "B_wqkv": _B_in["wqkv"],
        "B_wo": _B_in["wo"],
    }

def reference(A_x, A_wqkv, A_wo, B_x, B_wqkv, B_wo):
    def _A_ref(x, wqkv, wo):
        B, S, D = x.shape
        H = 32; Dh = D // H
        W, dil = 8, 2
        qkv = (lambda x, *d: x.transpose(*d))((x @ wqkv).reshape(B, S, 3, H, Dh), 2, 0, 3, 1, 4)
        q, k, v = qkv[0], qkv[1], qkv[2]
        scale = Dh ** -0.5
        pos = jnp.arange(S)
        off = jnp.arange(W) * dil
        idx = pos[:, None] - off[None, :]
        mask = idx >= 0
        idx_c = jnp.where(mask, idx, 0).reshape(-1)
        kg = k[:, :, idx_c, :].reshape(B, H, S, W, Dh)
        vg = v[:, :, idx_c, :].reshape(B, H, S, W, Dh)
        logits = jnp.einsum("bhsd,bhswd->bhsw", q, kg) * scale
        logits = jnp.where(mask[None, None, :, :], logits, -1e9)
        attn = _softmax(logits, axis=-1)
        o = jnp.einsum("bhsw,bhswd->bhsd", attn, vg)
        return (lambda x, *d: x.transpose(*d))(o, 0, 2, 1, 3).reshape(B, S, D) @ wo

    def _B_ref(x, wqkv, wo):
        B, S, D = x.shape
        H = 32; Dh = D // H; W = 256
        qkv = (lambda x, *d: x.transpose(*d))((x @ wqkv).reshape(B, S, 3, H, Dh), 2, 0, 3, 1, 4)
        q, k, v = qkv[0], qkv[1], qkv[2]
        scores = jnp.einsum("bhqd,bhkd->bhqk", q, k) * (Dh ** -0.5)
        idx = jnp.arange(S)
        mask = (idx[:, None] - idx[None, :] >= 0) & (idx[:, None] - idx[None, :] < W)
        scores = jnp.where(mask[None, None], scores, -1e9)
        p = _softmax(scores, axis=-1)
        o = jnp.einsum("bhqk,bhkd->bhqd", p, v)
        return (lambda x, *d: x.transpose(*d))(o, 0, 2, 1, 3).reshape(B, S, D) @ wo

    a = _A_ref(A_x, A_wqkv, A_wo)
    b = _B_ref(B_x, B_wqkv, B_wo)
    return jnp.concatenate([a, b], axis=-1)
```

```python
import functools

import numpy as np
import jax
import jax.numpy as jnp
from jax import lax
import jax.experimental.pallas as pl
import jax.experimental.pallas.tpu as pltpu

S, D, DH = 2048, 1024, 32
T = 128
NT = S // T
G = D // 128
f32, bf16, u32 = jnp.float32, jnp.bfloat16, jnp.uint32
NEG = -1e30
QSCALE = float(DH ** -0.5 * np.log2(np.e))
NT_DIMS = (((1,), (1,)), ((), ()))
ROW_OF_W = (0, 4, 2, 6, 1, 5, 3, 7)

N_FIRST = 2
LOOK = 4
PERM_DIST = 3


def _tables():
    r = np.arange(128)[:, None]
    c = np.arange(128)[None, :]
    b0 = np.where(r > c, 0.0, NEG)
    b2 = np.where(r <= c, 0.0, NEG)
    ba = np.zeros((8, 8, 128))
    for u in range(8):
        for row in range(8):
            if u < ROW_OF_W[row]:
                ba[u, row, 0:2] = NEG
    return np.concatenate([b0, b2, ba.reshape(64, 128)], axis=0).astype(np.float32)


def _rcp(l):
    r = pl.reciprocal(l, approx=True)
    return r * (2.0 - l * r)


def _red(x, op):
    acc = x[0:8]
    for j in range(1, x.shape[0] // 8):
        acc = op(acc, x[8 * j:8 * j + 8])
    return acc


def _kernel(zero_ref, tab_ref, xa_hbm, wa_hbm, woa_hbm, xb_hbm, wb_hbm, wob_hbm, out_hbm,
            xbu, xau, xap, wbu, wau, wobu, woau,
            qb, kb, vtb, ob,
            qta, kta, vta, oau,
            s0buf, s1buf, obuf,
            sem_xb, sem_xa, sem_wb, sem_oth, osem):
    zero = zero_ref[0]

    def colblk(hbm, n, r0=0, nr=None):
        nr = hbm.shape[0] if nr is None else nr
        c0 = n * 128 if isinstance(n, int) else pl.multiple_of(n * 128, 128)
        r0 = r0 if isinstance(r0, int) else pl.multiple_of(r0, 256)
        return hbm.at[pl.ds(r0, nr), pl.ds(c0, 128)]

    def xb_copy(j, kt):
        w0 = j * 128 if isinstance(j, int) else pl.multiple_of(j * 128, 128)
        return pltpu.make_async_copy(colblk(xb_hbm, kt, j * 256, 256),
                                     xbu.at[kt, pl.ds(w0, 128)].bitcast(bf16), sem_xb.at[j])

    def w_copy(hbm, dst, n, sem):
        return pltpu.make_async_copy(colblk(hbm, n), dst.at[n].bitcast(bf16), sem)

    worder = [t * G + g for g in range(G) for t in range(3)]

    def wb_copy(pos):
        n = worder[pos]
        return w_copy(wb_hbm, wbu, n, sem_xb.at[0] if pos < N_FIRST else sem_wb.at[n])

    def xa_copy(kt):
        return pltpu.make_async_copy(colblk(xa_hbm, kt), xau.at[kt].bitcast(bf16), sem_xa.at[kt])

    def wa_copy(n):
        return w_copy(wa_hbm, wau, n, sem_oth.at[0])

    def wob_copy(n):
        return w_copy(wob_hbm, wobu, n, sem_oth.at[1])

    def woa_copy(n):
        return w_copy(woa_hbm, woau, n, sem_oth.at[2])

    for kt in range(G):
        xb_copy(0, kt).start()
    for pos in range(LOOK):
        wb_copy(pos).start()

    for g in range(G):
        kb[g, 0:256, :] = jnp.zeros((256, 128), bf16)
    vtb[0:2] = jnp.zeros((2, D, 128), bf16)

    lane64 = lax.broadcasted_iota(jnp.int32, (64, 128), 1)
    head_mask = [jnp.where((lane64 >= 32 * h) & (lane64 < 32 * h + 32), u32(0xFFFFFFFF), u32(0))
                 for h in range(4)]
    sub8 = lax.broadcasted_iota(jnp.int32, (8, 128), 0)

    def rowmask(rows_):
        bits = sum(1 << r for r in rows_)
        return ((jnp.int32(bits) >> sub8) & 1) == 1

    def b16(x):
        return pltpu.bitcast(x, bf16)

    def wrows(i, n=64):
        return pl.ds(pl.multiple_of(i * 64, 8), n)

    def rows(i, n=T, off=0):
        return pl.ds(pl.multiple_of(i * T + off, 16), n)

    def tie(v, tok, r0=0):
        if tok is None:
            return v
        zvec = jnp.full((8, 128), zero, jnp.int32).astype(u32)
        parts = [v[0:r0]] if r0 else []
        parts.append(v[r0:r0 + 8] | (tok & zvec))
        if r0 + 8 < v.shape[0]:
            parts.append(v[r0 + 8:])
        return jnp.concatenate(parts, axis=0)

    qb_u, kb_u, vtb_u, ob_u = qb.bitcast(u32), kb.bitcast(u32), vtb.bitcast(u32), ob.bitcast(u32)

    def proj_b(i, g, t, tok=None):
        m = 2 * T
        x = jnp.concatenate([b16(xbu[kt, wrows(i, m // 2), :]) for kt in range(G)], axis=1)
        r = jnp.dot(x, b16(tie(wbu[t * G + g], tok)), preferred_element_type=f32)
        if t == 0:
            qb[g, rows(i, m), :] = (r * QSCALE).astype(bf16)
        elif t == 1:
            kb[g, rows(i, m, 256), :] = r.astype(bf16)
        else:
            for j in range(2):
                vtb[i + 2 + j, g * 128:(g + 1) * 128, :] = r[j * T:(j + 1) * T].astype(bf16).T

    def xa_permute(kt, u):
        xap[u, kt] = xau[kt, pl.ds(u, 64, stride=16), :]

    def proj_a(u, g, t):
        x = jnp.concatenate([b16(xap[u, kt]) for kt in range(G)], axis=1)
        r = jnp.dot(x, b16(wau[t * G + g]), preferred_element_type=f32)
        fr = slice(g * 128, (g + 1) * 128)
        if t == 0:
            qta[u, fr, :] = (r * QSCALE).T
        else:
            dst = kta if t == 1 else vta
            rt = r.T
            dst[u + 8, fr, :] = rt
            dst[jnp.where(u >= 9, u - 8, 0), fr, :] = pltpu.roll(rt, 2, axis=1)

    sbufs = (s0buf, s1buf)

    def att_b_group(i, g, fill):
        sb = sbufs[g % 2]
        q_u = qb_u[g, wrows(i), :]
        kw = b16(kb_u[g, wrows(i, 192), :])
        b0 = jnp.where(i >= 2, 0.0, NEG).astype(f32)
        b1 = jnp.where(i >= 1, 0.0, NEG).astype(f32)
        ms = []
        for h in range(4):
            s = lax.dot_general(kw, b16(q_u & head_mask[h]), NT_DIMS, preferred_element_type=f32)
            s0 = s[0:128] + tab_ref[0:128]
            s1 = s[128:256]
            s2 = s[256:384] + tab_ref[128:256]
            sb[h, 0:128] = s0
            sb[h, 128:256] = s1
            sb[h, 256:384] = s2
            m8 = jnp.maximum(jnp.maximum(_red(s0, jnp.maximum) + b0, _red(s1, jnp.maximum) + b1),
                             _red(s2, jnp.maximum))
            m = jnp.max(m8, axis=0, keepdims=True)
            ms.append((m - b0, m - b1, m))
        fill[0]()
        outs = []
        for h in range(4):
            ps = []
            l8 = None
            for t in range(3):
                p = jnp.exp2(sb[zero + h, t * 128:(t + 1) * 128] - ms[h][t])
                lp = _red(p, jnp.add)
                l8 = lp if l8 is None else l8 + lp
                ps.append(p)
            l = jnp.sum(l8, axis=0, keepdims=True)
            p = jnp.concatenate(ps, axis=0).astype(bf16)
            r0 = g * 64 + 16 * h
            vt = jnp.concatenate([b16(vtb_u[i + t, r0:r0 + 16, :]) for t in range(3)], axis=1)
            outs.append(jnp.dot(vt, p, preferred_element_type=f32) * _rcp(l))
            if h == 1:
                fill[1]()
        ob[g, rows(i), :] = jnp.concatenate(outs, axis=0).astype(bf16).T
        fill[2]()

    def reduce8(part):
        def comb(a, b, mask, shift):
            return jnp.where(mask, a, b) + pltpu.roll(jnp.where(mask, b, a), shift, axis=0)

        def s1(a, b, o):
            return comb(a, b, rowmask([(o + j) % 8 for j in range(4)]), 4)

        def s2(a, b, o):
            return comb(a, b, rowmask([(o + j) % 8 for j in (0, 1, 4, 5)]), 6)
        c = s2(s1(part[0], part[1], 0), s1(part[2], part[3], 2), 0)
        d = s2(s1(part[4], part[5], 1), s1(part[6], part[7], 3), 1)
        return comb(c, d, rowmask([0, 2, 4, 6]), 7)

    def att_a_head(u, h, bias):
        r = slice(32 * h, 32 * h + 32)
        q = qta[u, r, :]
        part = []
        for w in range(8):
            pr = q * kta[u + 8 - w, r, :]
            part.append((pr[0:8] + pr[8:16]) + (pr[16:24] + pr[24:32]))
        logits = reduce8(part) + bias
        e = jnp.exp2(logits - jnp.max(logits, axis=0, keepdims=True))
        p = e * _rcp(jnp.sum(e, axis=0, keepdims=True))
        o = None
        for w in range(8):
            rw = ROW_OF_W[w]
            t = jnp.broadcast_to(p[rw:rw + 1, :], (32, 128)) * vta[u + 8 - w, r, :]
            o = t if o is None else o + t
        return o

    def att_a_group(u, g, bias):
        ot = jnp.concatenate([att_a_head(u, 4 * g + h, bias) for h in range(4)], axis=0)
        res = pltpu.bitcast(ot.astype(bf16).T, u32)
        oau[g, pl.ds(u, 64, stride=16), :] = res
        return res[56:64]

    def out_piece(lhs, wou, slot, n, w):
        wt = jnp.concatenate([b16(wou[n * (w // 128) + j]) for j in range(w // 128)], axis=1)
        obuf[slot, :, n * w:(n + 1) * w] = jnp.dot(lhs, wt, preferred_element_type=f32).astype(bf16)

    def out_copy(slot, i, half):
        return pltpu.make_async_copy(obuf.at[slot], out_hbm.at[rows(i), pl.ds(half * D, D)], osem.at[slot])

    def start_a(j):
        xa_copy(j).start()
        for t in range(3):
            wa_copy(t * G + j).start()

    for kt in range(G):
        xb_copy(0, kt).wait()
    for pos in range(N_FIRST):
        wb_copy(pos).wait()
    for pos in range(3 * G):
        if pos >= N_FIRST:
            wb_copy(pos).wait()
        if pos + LOOK < 3 * G:
            wb_copy(pos + LOOK).start()
        elif pos + LOOK == 3 * G:
            for kt in range(G):
                xb_copy(1, kt).start()
            start_a(0)
            start_a(1)
        proj_b(0, pos // 3, pos % 3)

    def phase1(j, carry):
        @pl.when(j < 7)
        def _():
            for kt in range(G):
                xb_copy(j + 1, kt).start()
            start_a(j + 1)
        for kt in range(G):
            xb_copy(j, kt).wait()
        xa_copy(j - 1).wait()
        toks = []
        for g in range(G):
            for t in ((0, 1, 2) if g < G - 1 else (2, 1, 0)):
                pos = 3 * g + t
                if pos < NT:
                    xa_permute(j - 1, pos)
                    toks.append(xap[zero + pos, j - 1, 0:8, :])
                tok = toks[pos - PERM_DIST] if PERM_DIST <= pos < NT + PERM_DIST else None
                proj_b(2 * j, g, t, tok)
        return carry
    lax.fori_loop(1, 8, phase1, 0)

    for n in range(3 * G):
        wa_copy(n).wait()
    for n in range(G):
        wob_copy(n).start()
    for n in range(G):
        woa_copy(n).start()
    xa_copy(7).wait()
    for u in range(NT):
        xa_permute(7, u)

    def phase2(i2, carry):
        for sub in range(2):
            i = 2 * i2 + sub
            for g in range(G):
                order = (2, 1, 0) if (sub == 1 and g == G - 1) else (0, 1, 2)
                att_b_group(i, g, [functools.partial(proj_a, i, g, t) for t in order])
        return carry
    lax.fori_loop(0, NT // 2, phase2, 0)

    for n in range(G):
        wob_copy(n).wait()

    def phase3(i2, carry):
        s0 = 2 * (i2 % 2)

        @pl.when(i2 >= 2)
        def _():
            for sub in range(2):
                out_copy(s0 + sub, 0, 1).wait()
        toks = []
        for sub in range(2):
            i = 2 * i2 + sub
            bias = tab_ref[pl.ds(pl.multiple_of(256 + 8 * jnp.minimum(i, 7), 8), 8), :]
            for g in range(G):
                tok = toks[-1] if toks else None
                lhs = jnp.concatenate(
                    [b16(tie(ob_u[gg, wrows(i), :], tok if gg == 3 else None, 56)) for gg in range(G)], axis=1)
                out_piece(lhs, wobu, s0 + sub, g, 128)
                toks.append(att_a_group(i, g, bias))
            out_copy(s0 + sub, i, 1).start()
        return carry
    lax.fori_loop(0, NT // 2, phase3, 0)
    for slot in range(4):
        out_copy(slot, 0, 1).wait()

    for n in range(G):
        woa_copy(n).wait()

    def phase4(i2, carry):
        s0 = 2 * (i2 % 2)

        @pl.when(i2 >= 2)
        def _():
            for sub in range(2):
                out_copy(s0 + sub, 0, 0).wait()
        for sub in range(2):
            i = 2 * i2 + sub
            for n in range(4):
                lhs = jnp.concatenate([b16(oau[g, wrows(i), :]) for g in range(G)], axis=1)
                out_piece(lhs, woau, s0 + sub, n, 256)
            out_copy(s0 + sub, i, 0).start()
        return carry
    lax.fori_loop(0, NT // 2, phase4, 0)
    for slot in range(4):
        out_copy(slot, 0, 0).wait()


@jax.jit
def pallas_concat_heads__sliding_local_dilated__sliding_block__prompt_kernel(A_x, A_wqkv, A_wo, B_x, B_wqkv, B_wo):
    zero = jnp.zeros((1,), jnp.int32)
    tab = jnp.asarray(_tables())
    vmem = pltpu.VMEM
    dma = pltpu.SemaphoreType.DMA
    scratch = [
        vmem((G, S // 2, 128), u32), vmem((G, S // 2, 128), u32), vmem((NT, G, 64, 128), u32),
        vmem((3 * G, D // 2, 128), u32), vmem((3 * G, D // 2, 128), u32),
        vmem((G, D // 2, 128), u32), vmem((G, D // 2, 128), u32),
        vmem((G, S, 128), bf16), vmem((G, S + 256, 128), bf16), vmem((NT + 2, D, 128), bf16),
        vmem((G, S, 128), bf16),
        vmem((NT, D, 128), f32), vmem((NT + 8, D, 128), f32), vmem((NT + 8, D, 128), f32),
        vmem((G, S // 2, 128), u32),
        vmem((4, 384, 128), f32), vmem((4, 384, 128), f32),
        vmem((4, T, D), bf16),
        dma((8,)), dma((8,)), dma((3 * G,)), dma((3,)), dma((4,)),
    ]
    any_spec = pl.BlockSpec(memory_space=pl.ANY)
    out = pl.pallas_call(
        _kernel,
        grid_spec=pltpu.PrefetchScalarGridSpec(
            num_scalar_prefetch=1,
            grid=(1,),
            in_specs=[pl.BlockSpec((320, 128), lambda i, z: (0, 0))] + [any_spec] * 6,
            out_specs=any_spec,
            scratch_shapes=scratch,
        ),
        out_shape=jax.ShapeDtypeStruct((S, 2 * D), bf16),
        compiler_params=pltpu.CompilerParams(
            vmem_limit_bytes=110 * 1024 * 1024,
            flags={"XLA_TPU_RESCHEDULE_DMA_DONES": True},
        ),
        name="fused_attn",
    )(zero, tab, A_x.reshape(S, D), A_wqkv, A_wo, B_x.reshape(S, D), B_wqkv, B_wo)
    return out.reshape(1, S, 2 * D)
```

```python
import functools

import numpy as np
import jax
import jax.numpy as jnp
from jax import lax
import jax.experimental.pallas as pl
import jax.experimental.pallas.tpu as pltpu

S, D, DH = 2048, 1024, 32
T = 128
NT = S // T
G = D // 128
f32, bf16, u32 = jnp.float32, jnp.bfloat16, jnp.uint32
NEG = -1e30
QSCALE = float(DH ** -0.5 * np.log2(np.e))
NT_DIMS = (((1,), (1,)), ((), ()))
ROW_OF_W = (0, 4, 2, 6, 1, 5, 3, 7)

N_FIRST = 2
LOOK = 4
PERM_DIST = 3


def _tables():
    r = np.arange(128)[:, None]
    c = np.arange(128)[None, :]
    b0 = np.where(r > c, 0.0, NEG)
    b2 = np.where(r <= c, 0.0, NEG)
    ba = np.zeros((8, 8, 128))
    for u in range(8):
        for row in range(8):
            if u < ROW_OF_W[row]:
                ba[u, row, 0:2] = NEG
    return np.concatenate([b0, b2, ba.reshape(64, 128)], axis=0).astype(np.float32)


def _rcp(l):
    r = pl.reciprocal(l, approx=True)
    return r * (2.0 - l * r)


def _red(x, op):
    acc = x[0:8]
    for j in range(1, x.shape[0] // 8):
        acc = op(acc, x[8 * j:8 * j + 8])
    return acc


def _kernel(zero_hbm, tab_hbm, xa_hbm, wa_hbm, woa_hbm, xb_hbm, wb_hbm, wob_hbm, out_hbm,
            xbu, xau, xap, wbu, wau, wobu, woau,
            qb, kb, vtb, ob,
            qta, kta, vta, oau,
            s0buf, s1buf, obuf, zero_ref, tab_ref,
            sem_xb, sem_xa, sem_wb, sem_oth, osem):
    zero_cp = pltpu.make_async_copy(zero_hbm, zero_ref, sem_oth.at[3])
    tab_cp = pltpu.make_async_copy(tab_hbm, tab_ref, sem_oth.at[4])

    def colblk(hbm, n, r0=0, nr=None):
        nr = hbm.shape[0] if nr is None else nr
        c0 = n * 128 if isinstance(n, int) else pl.multiple_of(n * 128, 128)
        r0 = r0 if isinstance(r0, int) else pl.multiple_of(r0, 256)
        return hbm.at[pl.ds(r0, nr), pl.ds(c0, 128)]

    def xb_copy(j, kt):
        w0 = j * 128 if isinstance(j, int) else pl.multiple_of(j * 128, 128)
        return pltpu.make_async_copy(colblk(xb_hbm, kt, j * 256, 256),
                                     xbu.at[kt, pl.ds(w0, 128)].bitcast(bf16), sem_xb.at[j])

    def w_copy(hbm, dst, n, sem):
        return pltpu.make_async_copy(colblk(hbm, n), dst.at[n].bitcast(bf16), sem)

    worder = [t * G + g for g in range(G) for t in range(3)]

    def wb_copy(pos):
        n = worder[pos]
        return w_copy(wb_hbm, wbu, n, sem_xb.at[0] if pos < N_FIRST else sem_wb.at[n])

    def xa_copy(kt):
        return pltpu.make_async_copy(colblk(xa_hbm, kt), xau.at[kt].bitcast(bf16), sem_xa.at[kt])

    def wa_copy(n):
        return w_copy(wa_hbm, wau, n, sem_oth.at[0])

    def wob_copy(n):
        return w_copy(wob_hbm, wobu, n, sem_oth.at[1])

    def woa_copy(n):
        return w_copy(woa_hbm, woau, n, sem_oth.at[2])

    for kt in range(G):
        xb_copy(0, kt).start()
    for pos in range(LOOK):
        wb_copy(pos).start()
    zero_cp.start()

    for g in range(G):
        kb[g, 0:256, :] = jnp.zeros((256, 128), bf16)
    vtb[0:2] = jnp.zeros((2, D, 128), bf16)

    lane64 = lax.broadcasted_iota(jnp.int32, (64, 128), 1)
    head_mask = [jnp.where((lane64 >= 32 * h) & (lane64 < 32 * h + 32), u32(0xFFFFFFFF), u32(0))
                 for h in range(4)]
    sub8 = lax.broadcasted_iota(jnp.int32, (8, 128), 0)

    def rowmask(rows_):
        bits = sum(1 << r for r in rows_)
        return ((jnp.int32(bits) >> sub8) & 1) == 1

    def b16(x):
        return pltpu.bitcast(x, bf16)

    def wrows(i, n=64):
        return pl.ds(pl.multiple_of(i * 64, 8), n)

    def rows(i, n=T, off=0):
        return pl.ds(pl.multiple_of(i * T + off, 16), n)

    def tie(v, tok, r0=0):
        if tok is None:
            return v
        zvec = jnp.full((8, 128), zero, jnp.int32).astype(u32)
        parts = [v[0:r0]] if r0 else []
        parts.append(v[r0:r0 + 8] | (tok & zvec))
        if r0 + 8 < v.shape[0]:
            parts.append(v[r0 + 8:])
        return jnp.concatenate(parts, axis=0)

    qb_u, kb_u, vtb_u, ob_u = qb.bitcast(u32), kb.bitcast(u32), vtb.bitcast(u32), ob.bitcast(u32)

    def proj_b(i, g, t, tok=None):
        m = 2 * T
        x = jnp.concatenate([b16(xbu[kt, wrows(i, m // 2), :]) for kt in range(G)], axis=1)
        r = jnp.dot(x, b16(tie(wbu[t * G + g], tok)), preferred_element_type=f32)
        if t == 0:
            qb[g, rows(i, m), :] = (r * QSCALE).astype(bf16)
        elif t == 1:
            kb[g, rows(i, m, 256), :] = r.astype(bf16)
        else:
            for j in range(2):
                vtb[i + 2 + j, g * 128:(g + 1) * 128, :] = r[j * T:(j + 1) * T].astype(bf16).T

    def xa_permute(kt, u):
        xap[u, kt] = xau[kt, pl.ds(u, 64, stride=16), :]

    def proj_a(u, g, t):
        x = jnp.concatenate([b16(xap[u, kt]) for kt in range(G)], axis=1)
        r = jnp.dot(x, b16(wau[t * G + g]), preferred_element_type=f32)
        fr = slice(g * 128, (g + 1) * 128)
        if t == 0:
            qta[u, fr, :] = (r * QSCALE).T
        else:
            dst = kta if t == 1 else vta
            rt = r.T
            dst[u + 8, fr, :] = rt
            dst[jnp.where(u >= 9, u - 8, 0), fr, :] = pltpu.roll(rt, 2, axis=1)

    sbufs = (s0buf, s1buf)

    def att_b_group(i, g, fill):
        sb = sbufs[g % 2]
        q_u = qb_u[g, wrows(i), :]
        kw = b16(kb_u[g, wrows(i, 192), :])
        b0 = jnp.where(i >= 2, 0.0, NEG).astype(f32)
        b1 = jnp.where(i >= 1, 0.0, NEG).astype(f32)
        ms = []
        for h in range(4):
            s = lax.dot_general(kw, b16(q_u & head_mask[h]), NT_DIMS, preferred_element_type=f32)
            s0 = s[0:128] + tab_ref[0:128]
            s1 = s[128:256]
            s2 = s[256:384] + tab_ref[128:256]
            sb[h, 0:128] = s0
            sb[h, 128:256] = s1
            sb[h, 256:384] = s2
            m8 = jnp.maximum(jnp.maximum(_red(s0, jnp.maximum) + b0, _red(s1, jnp.maximum) + b1),
                             _red(s2, jnp.maximum))
            m = jnp.max(m8, axis=0, keepdims=True)
            ms.append((m - b0, m - b1, m))
        fill[0]()
        outs = []
        for h in range(4):
            ps = []
            l8 = None
            for t in range(3):
                p = jnp.exp2(sb[zero + h, t * 128:(t + 1) * 128] - ms[h][t])
                lp = _red(p, jnp.add)
                l8 = lp if l8 is None else l8 + lp
                ps.append(p)
            l = jnp.sum(l8, axis=0, keepdims=True)
            p = jnp.concatenate(ps, axis=0).astype(bf16)
            r0 = g * 64 + 16 * h
            vt = jnp.concatenate([b16(vtb_u[i + t, r0:r0 + 16, :]) for t in range(3)], axis=1)
            outs.append(jnp.dot(vt, p, preferred_element_type=f32) * _rcp(l))
            if h == 0:
                fill[1]()
        ob[g, rows(i), :] = jnp.concatenate(outs, axis=0).astype(bf16).T
        fill[2]()

    def reduce8(part):
        def comb(a, b, mask, shift):
            return jnp.where(mask, a, b) + pltpu.roll(jnp.where(mask, b, a), shift, axis=0)

        def s1(a, b, o):
            return comb(a, b, rowmask([(o + j) % 8 for j in range(4)]), 4)

        def s2(a, b, o):
            return comb(a, b, rowmask([(o + j) % 8 for j in (0, 1, 4, 5)]), 6)
        c = s2(s1(part[0], part[1], 0), s1(part[2], part[3], 2), 0)
        d = s2(s1(part[4], part[5], 1), s1(part[6], part[7], 3), 1)
        return comb(c, d, rowmask([0, 2, 4, 6]), 7)

    def att_a_head(u, h, bias):
        r = slice(32 * h, 32 * h + 32)
        q = qta[u, r, :]
        part = []
        for w in range(8):
            pr = q * kta[u + 8 - w, r, :]
            part.append((pr[0:8] + pr[8:16]) + (pr[16:24] + pr[24:32]))
        logits = reduce8(part) + bias
        e = jnp.exp2(logits - jnp.max(logits, axis=0, keepdims=True))
        p = e * _rcp(jnp.sum(e, axis=0, keepdims=True))
        o = None
        for w in range(8):
            rw = ROW_OF_W[w]
            t = jnp.broadcast_to(p[rw:rw + 1, :], (32, 128)) * vta[u + 8 - w, r, :]
            o = t if o is None else o + t
        return o

    def att_a_group(u, g, bias):
        ot = jnp.concatenate([att_a_head(u, 4 * g + h, bias) for h in range(4)], axis=0)
        res = pltpu.bitcast(ot.astype(bf16).T, u32)
        oau[g, pl.ds(u, 64, stride=16), :] = res
        return res[56:64]

    def out_piece(lhs, wou, slot, n, w):
        wt = jnp.concatenate([b16(wou[n * (w // 128) + j]) for j in range(w // 128)], axis=1)
        obuf[slot, :, n * w:(n + 1) * w] = jnp.dot(lhs, wt, preferred_element_type=f32).astype(bf16)

    def out_copy(slot, i, half):
        return pltpu.make_async_copy(obuf.at[slot], out_hbm.at[rows(i), pl.ds(half * D, D)], osem.at[slot])

    def start_a(j):
        xa_copy(j).start()
        for t in range(3):
            wa_copy(t * G + j).start()

    for kt in range(G):
        xb_copy(0, kt).wait()
    for pos in range(N_FIRST):
        wb_copy(pos).wait()
    for pos in range(3 * G):
        if pos >= N_FIRST:
            wb_copy(pos).wait()
        if pos + LOOK < 3 * G:
            wb_copy(pos + LOOK).start()
        elif pos + LOOK == 3 * G:
            for kt in range(G):
                xb_copy(1, kt).start()
            start_a(0)
            start_a(1)
        proj_b(0, pos // 3, pos % 3)

    tab_cp.start()
    zero_cp.wait()
    zero = zero_ref[0]

    def phase1(j, carry):
        @pl.when(j < 7)
        def _():
            for kt in range(G):
                xb_copy(j + 1, kt).start()
            start_a(j + 1)
        for kt in range(G):
            xb_copy(j, kt).wait()
        xa_copy(j - 1).wait()
        toks = []
        for g in range(G):
            for t in ((0, 1, 2) if g < G - 1 else (2, 1, 0)):
                pos = 3 * g + t
                if pos < NT:
                    xa_permute(j - 1, pos)
                    toks.append(xap[zero + pos, j - 1, 0:8, :])
                tok = toks[pos - PERM_DIST] if PERM_DIST <= pos < NT + PERM_DIST else None
                proj_b(2 * j, g, t, tok)
        return carry
    lax.fori_loop(1, 8, phase1, 0)

    tab_cp.wait()
    for n in range(3 * G):
        wa_copy(n).wait()
    for n in range(G):
        wob_copy(n).start()
    for n in range(G):
        woa_copy(n).start()
    xa_copy(7).wait()
    for u in range(NT):
        xa_permute(7, u)

    def phase2(i2, carry):
        for sub in range(2):
            i = 2 * i2 + sub
            for g in range(G):
                att_b_group(i, g, [functools.partial(proj_a, i, g, t) for t in (2, 1, 0)])
        return carry
    lax.fori_loop(0, NT // 2, phase2, 0)

    for n in range(G):
        wob_copy(n).wait()

    def phase3(i2, carry):
        s0 = 2 * (i2 % 2)

        @pl.when(i2 >= 2)
        def _():
            for sub in range(2):
                out_copy(s0 + sub, 0, 1).wait()
        toks = []
        for sub in range(2):
            i = 2 * i2 + sub
            bias = tab_ref[pl.ds(pl.multiple_of(256 + 8 * jnp.minimum(i, 7), 8), 8), :]
            for g in range(G):
                tok = toks[-1] if toks else None
                lhs = jnp.concatenate(
                    [b16(tie(ob_u[gg, wrows(i), :], tok if gg == 3 else None, 56)) for gg in range(G)], axis=1)
                out_piece(lhs, wobu, s0 + sub, g, 128)
                toks.append(att_a_group(i, g, bias))
            out_copy(s0 + sub, i, 1).start()
        return carry
    lax.fori_loop(0, NT // 2, phase3, 0)
    for slot in range(4):
        out_copy(slot, 0, 1).wait()

    for n in range(G):
        woa_copy(n).wait()

    def phase4(i2, carry):
        s0 = 2 * (i2 % 2)

        @pl.when(i2 >= 2)
        def _():
            for sub in range(2):
                out_copy(s0 + sub, 0, 0).wait()
        for sub in range(2):
            i = 2 * i2 + sub
            for n in range(4):
                lhs = jnp.concatenate([b16(oau[g, wrows(i), :]) for g in range(G)], axis=1)
                out_piece(lhs, woau, s0 + sub, n, 256)
                pltpu.make_async_copy(obuf.at[s0 + sub, :, pl.ds(n * 256, 256)],
                                      out_hbm.at[rows(i), pl.ds(n * 256, 256)], osem.at[s0 + sub]).start()
        return carry
    lax.fori_loop(0, NT // 2, phase4, 0)
    for slot in range(4):
        out_copy(slot, 0, 0).wait()


@jax.jit
def pallas_concat_heads__sliding_local_dilated__sliding_block__prompt_kernel(A_x, A_wqkv, A_wo, B_x, B_wqkv, B_wo):
    zero = jnp.zeros((1,), jnp.int32)
    tab = jnp.asarray(_tables())
    vmem = pltpu.VMEM
    dma = pltpu.SemaphoreType.DMA
    scratch = [
        vmem((G, S // 2, 128), u32), vmem((G, S // 2, 128), u32), vmem((NT, G, 64, 128), u32),
        vmem((3 * G, D // 2, 128), u32), vmem((3 * G, D // 2, 128), u32),
        vmem((G, D // 2, 128), u32), vmem((G, D // 2, 128), u32),
        vmem((G, S, 128), bf16), vmem((G, S + 256, 128), bf16), vmem((NT + 2, D, 128), bf16),
        vmem((G, S, 128), bf16),
        vmem((NT, D, 128), f32), vmem((NT + 8, D, 128), f32), vmem((NT + 8, D, 128), f32),
        vmem((G, S // 2, 128), u32),
        vmem((4, 384, 128), f32), vmem((4, 384, 128), f32),
        vmem((4, T, D), bf16),
        pltpu.SMEM((1,), jnp.int32), vmem((320, 128), f32),
        dma((8,)), dma((8,)), dma((3 * G,)), dma((5,)), dma((4,)),
    ]
    any_spec = pl.BlockSpec(memory_space=pl.ANY)
    out = pl.pallas_call(
        _kernel,
        in_specs=[any_spec] * 8,
        out_specs=any_spec,
        scratch_shapes=scratch,
        out_shape=jax.ShapeDtypeStruct((S, 2 * D), bf16),
        compiler_params=pltpu.CompilerParams(
            vmem_limit_bytes=110 * 1024 * 1024,
            flags={"XLA_TPU_RESCHEDULE_DMA_DONES": True},
        ),
        name="fused_attn",
    )(zero, tab, A_x.reshape(S, D), A_wqkv, A_wo, B_x.reshape(S, D), B_wqkv, B_wo)
    return out.reshape(1, S, 2 * D)
```
